```python
import jax
import jax.numpy as jnp

def _softmax(x, axis=-1):
    return jax.nn.softmax(x, axis=axis)

def _gelu(x):
    return jax.nn.gelu(x, approximate=True)

def _silu(x):
    return jax.nn.silu(x)

def _sigmoid(x):
    return jax.nn.sigmoid(x)

def _layernorm(x, axis=-1, eps=1e-05):
    m = jnp.mean(x, axis=axis, keepdims=True)
    v = jnp.var(x, axis=axis, keepdims=True)
    return (x - m) / jnp.sqrt(v + eps)

def _scatter_add(tgt, idx, src, axis=0):
    return tgt.at[idx].add(src)

def _segment_sum(src, seg, n):
    return jax.ops.segment_sum(src, seg, n)

class _Rng:

    def __init__(self, key):
        self._k = key

    def _next(self):
        self._k, sub = jax.random.split(self._k)
        return sub

    def normal(self, shape):
        return jax.random.normal(self._next(), shape, dtype=jnp.bfloat16)

    def randint(self, lo, hi, shape):
        return jax.random.randint(self._next(), shape, lo, hi, dtype=jnp.int32)

    def uniform(self, shape, lo=0.0, hi=1.0):
        return jax.random.uniform(self._next(), shape, jnp.bfloat16, lo, hi)

    def permutation(self, n):
        return jax.random.permutation(self._next(), n)
kernel_name = 'interleave_layers__memory_aug_infini_attn__mixer_s_mlp__prompt'

def setup_inputs():
    _rng = _Rng(jax.random.key(int.from_bytes(__import__("os").urandom(4), "little")))
    _w = lambda a: (lambda t: t.astype(jnp.bfloat16) if jnp.issubdtype(t.dtype, jnp.floating) else t)(jnp.asarray(a))

    def _A_setup():
        B, S, D, H = (1, 2048, 1024, 32)
        N = 4
        L = max(1, S // N)
        sc = D ** (-0.5)
        return {'x': _w((lambda *s: _rng.normal(s) * 0.05)(B, N * L, D)), 'wq': _w((lambda *s: _rng.normal(s) * 0.05)(D, D) * sc), 'wk': _w((lambda *s: _rng.normal(s) * 0.05)(D, D) * sc), 'wv': _w((lambda *s: _rng.normal(s) * 0.05)(D, D) * sc), 'wo': _w((lambda *s: _rng.normal(s) * 0.05)(D, D) * sc), 'beta': _w((lambda *s: _rng.normal(s) * 0.05)(H))}
    _A_in = _A_setup()

    def _B_setup():
        B, S, D, F = (1, 2048, 1024, 3584)
        return {'x': _w((lambda *s: _rng.normal(s) * 0.05)(B, S, D)), 'w1': _w((lambda *s: _rng.normal(s) * 0.05)(D, D) * D ** (-0.5)), 'w2': _w((lambda *s: _rng.normal(s) * 0.05)(D, D) * D ** (-0.5)), 'w3': _w((lambda *s: _rng.normal(s) * 0.05)(D, F) * D ** (-0.5)), 'w4': _w((lambda *s: _rng.normal(s) * 0.05)(F, D) * F ** (-0.5))}
    _B_in = _B_setup()
    return {'A_x': _A_in['x'], 'A_wq': _A_in['wq'], 'A_wk': _A_in['wk'], 'A_wv': _A_in['wv'], 'A_wo': _A_in['wo'], 'A_beta': _A_in['beta'], 'B_x': _B_in['x'], 'B_w1': _B_in['w1'], 'B_w2': _B_in['w2'], 'B_w3': _B_in['w3'], 'B_w4': _B_in['w4']}

def reference(A_x, A_wq, A_wk, A_wv, A_wo, A_beta, B_x, B_w1, B_w2, B_w3, B_w4):

    def _A_ref(x, wq, wk, wv, wo, beta):
        B, S, D = x.shape
        H = 32
        Dh = D // H
        N = 4
        L = S // N
        q = (lambda x, *d: x.transpose(*d))((x @ wq).reshape(B, S, H, Dh), 0, 2, 1, 3).reshape(B, H, N, L, Dh)
        k = (lambda x, *d: x.transpose(*d))((x @ wk).reshape(B, S, H, Dh), 0, 2, 1, 3).reshape(B, H, N, L, Dh)
        v = (lambda x, *d: x.transpose(*d))((x @ wv).reshape(B, S, H, Dh), 0, 2, 1, 3).reshape(B, H, N, L, Dh)
        phi = lambda t: jnp.where(t > 0, t + 1.0, jnp.exp(t))
        scale = Dh ** (-0.5)
        ar = jnp.arange(L)
        mask = (lambda x, dt: x.astype(dt))(ar[:, None] < ar[None, :], x.dtype) * -1000000000.0
        g = _sigmoid(beta).reshape(1, H, 1, 1)
        M = jnp.einsum('bhd,bhe->bhde', q[:, :, 0, 0, :] * 0.0, q[:, :, 0, 0, :] * 0.0)
        z = q[:, :, 0, 0, :] * 0.0
        outs = []
        for s in range(N):
            qs, ks, vs = (q[:, :, s].copy(), k[:, :, s].copy(), v[:, :, s].copy())
            logits = jnp.einsum('bhqd,bhkd->bhqk', qs, ks) * scale + mask
            p = _softmax(logits, axis=-1)
            a_dot = jnp.einsum('bhqk,bhkd->bhqd', p, vs)
            pq = phi(qs)
            num = jnp.einsum('bhld,bhde->bhle', pq, M)
            den = jnp.einsum('bhld,bhd->bhl', pq, z)[..., None] + 1e-06
            a_mem = num / den
            o = g * a_mem + (1.0 - g) * a_dot
            outs.append(o)
            pk = phi(ks)
            M = M + jnp.einsum('bhld,bhle->bhde', pk, vs)
            z = z + jnp.einsum('bhld->bhd', pk)
        o = (lambda x, *d: x.transpose(*d))(jnp.stack(outs, 2).reshape(B, H, S, Dh), 0, 2, 1, 3).reshape(B, S, D)
        return o @ wo

    def _B_ref(x, w1, w2, w3, w4):
        B, S, D = x.shape
        h = _gelu(_layernorm(x, axis=-1) @ w1)
        c = D // 4
        g0 = jnp.pad(h[:, :, 0 * c:1 * c], ((0, 0), (1, 0), (0, 0)))[:, :S, :]
        g1 = jnp.pad(h[:, :, 1 * c:2 * c], ((0, 0), (0, 1), (0, 0)))[:, 1:, :]
        g2 = jnp.pad(h[:, :, 2 * c:3 * c], ((0, 0), (2, 0), (0, 0)))[:, :S, :]
        g3 = jnp.pad(h[:, :, 3 * c:], ((0, 0), (0, 2), (0, 0)))[:, 2:, :]
        hs = jnp.concatenate([g0, g1, g2, g3], axis=-1) @ w2
        x1 = x + hs
        h2 = _gelu(_layernorm(x1, axis=-1) @ w3) @ w4
        return x1 + h2
    x = A_x
    x = x + _A_ref(_layernorm(x, axis=-1), A_wq, A_wk, A_wv, A_wo, A_beta)
    x = x + _B_ref(_layernorm(x, axis=-1), B_w1, B_w2, B_w3, B_w4)
    x = x + _A_ref(_layernorm(x, axis=-1), A_wq, A_wk, A_wv, A_wo, A_beta)
    x = x + _B_ref(_layernorm(x, axis=-1), B_w1, B_w2, B_w3, B_w4)
    return x
```

```python
import functools
import math

import jax
import jax.numpy as jnp
from jax import lax
import jax.experimental.pallas as pl
import jax.experimental.pallas.tpu as pltpu

S, D, H, DH, NSEG, L, F = 2048, 1024, 32, 32, 4, 512, 3584
G = 8
LOG2E = 1.4426950408889634
QSCALE = DH ** -0.5 * LOG2E
NEG = -1e9 * LOG2E
BF = jnp.bfloat16
F32 = jnp.float32

NT = (((1,), (1,)), ((), ()))
NN = (((1,), (0,)), ((), ()))
TN = (((0,), (0,)), ((), ()))
TT = (((0,), (1,)), ((), ()))


def mm(a, b, dn=NN):
    return lax.dot_general(a, b, dn, preferred_element_type=F32)


def ln(x):
    m = jnp.mean(x, axis=-1, keepdims=True)
    d = x - m
    v = jnp.mean(d * d, axis=-1, keepdims=True)
    return d * lax.rsqrt(v + 1e-5)


def gelu(x):
    c0 = math.sqrt(2.0 / math.pi)
    u = x * (x * x * (c0 * 0.044715) + c0)
    hx = 0.5 * x
    return hx * jnp.tanh(u) + hx


def phi(t):
    return jnp.where(t > 0, t + 1.0, jnp.exp(t))


def kernel(x_hbm, wq_hbm, wk_hbm, wv_hbm, wo_hbm, beta_ref, w1_hbm, w2_hbm, w3_hbm, w4_hbm,
           out_hbm,
           wq, wk, wv, wo, w1, w2, w3, w4,
           xb, X, XF, XN, Q, PQ, K, PK, VT, OT, MT, Z, A, HB, Gt, bias, sems, osem):
    copies = {}
    order = [("x", x_hbm, xb), ("wq", wq_hbm, wq), ("wk", wk_hbm, wk), ("wv", wv_hbm, wv), ("wo", wo_hbm, wo),
             ("w1", w1_hbm, w1), ("w2", w2_hbm, w2), ("w3", w3_hbm, w3), ("w4", w4_hbm, w4)]
    for i, (n, src, dst) in enumerate(order):
        c = pltpu.make_async_copy(src, dst, sems.at[i])
        c.start()
        copies[n] = c

    r = lax.broadcasted_iota(jnp.int32, (128, 128), 0)
    c = lax.broadcasted_iota(jnp.int32, (128, 128), 1)
    bias[...] = jnp.where(r > c, NEG, 0.0).astype(F32)
    lane_head = lax.broadcasted_iota(jnp.int32, (64, 128), 1) // DH
    masks = [jnp.where(lane_head == h, -1, 0).astype(jnp.int32) for h in range(4)]
    blk = (lax.broadcasted_iota(jnp.int32, (128, 128), 0) // DH) == (lax.broadcasted_iota(jnp.int32, (128, 128), 1) // DH)

    b = beta_ref[...].astype(F32)
    gv = jax.nn.sigmoid(b)
    rr = lax.broadcasted_iota(jnp.int32, (H, H), 0)
    cc = lax.broadcasted_iota(jnp.int32, (H, H), 1)
    col = jnp.sum(jnp.where(rr == cc, jnp.broadcast_to(gv, (H, H)), 0.0), axis=1, keepdims=True)
    gb = jnp.broadcast_to(col, (H, 128))
    for h in range(H):
        Gt[h] = jnp.broadcast_to(gb[h:h + 1, :], (8, 128))

    copies["x"].wait()
    for s in range(NSEG):
        X[pl.ds(s * L, L), :] = xb[pl.ds(s * L, L), :].astype(F32)

    def a_group(s, g):
        r0 = pl.multiple_of(s * L, L)
        c0 = pl.multiple_of(g * 128, 128)
        xn = XN[pl.ds(r0, L), :]
        q = mm(xn, wq[:, pl.ds(c0, 128)])
        Q[...] = (q * QSCALE).astype(BF)
        PQ[...] = phi(q).astype(BF)
        k = mm(xn, wk[:, pl.ds(c0, 128)])
        K[...] = k.astype(BF)
        pk = phi(k)
        PK[...] = pk.astype(BF)
        zs = jnp.sum(pk, axis=0, keepdims=True)
        vt = mm(wv[:, pl.ds(c0, 128)], xn, TT)
        VT[...] = vt.astype(BF)

        mem = mm(A[g], PQ[...], NT)
        for hh in range(4):
            gh = Gt[g * 4 + hh]
            for i in range(4):
                kv = 128 * (i + 1)
                qh = pltpu.bitcast(pltpu.bitcast(Q[pl.ds(128 * i, 128), :], jnp.int32) & masks[hh], BF)
                st = mm(K[pl.ds(0, kv), :], qh, NT)
                if i > 0:
                    st = jnp.concatenate([st[:kv - 128], st[kv - 128:] + bias[...]], axis=0)
                else:
                    st = st + bias[...]
                m = jnp.max(st, axis=0, keepdims=True)
                p = jnp.exp2(st - m)
                l = jnp.sum(p, axis=0, keepdims=True)
                ot = mm(VT[pl.ds(32 * hh, 32), pl.ds(0, kv)], p.astype(BF))
                num = mem[40 * hh:40 * hh + 32, 128 * i:128 * (i + 1)]
                den = mem[40 * hh + 32:40 * hh + 40, 128 * i:128 * (i + 1)] + 1e-6
                g1 = gh[0:1, :]
                wd = (1.0 - g1) / l
                wm = g1 / den[0:1, :]
                o = ot * wd + num * wm
                OT[g, pl.ds(32 * hh, 32), pl.ds(128 * i, 128)] = o.astype(BF)
        mt = MT[g] + jnp.where(blk, mm(VT[...], PK[...]), 0.0)
        MT[g] = mt
        z = Z[g] + jnp.broadcast_to(zs, (8, 128))
        Z[g] = z
        lh = lax.broadcasted_iota(jnp.int32, (8, 128), 1) // DH
        parts = []
        for hh in range(4):
            parts.append(mt[32 * hh:32 * hh + 32, :])
            parts.append(jnp.where(lh == hh, z, 0.0))
        A[g] = jnp.concatenate(parts, axis=0).astype(BF)

    def a_out(s):
        r0 = pl.multiple_of(s * L, L)
        acc = jnp.zeros((L, D), F32)
        for g in range(G):
            acc = acc + mm(OT[g], wo[pl.ds(g * 128, 128), :], TN)
        X[pl.ds(r0, L), :] = X[pl.ds(r0, L), :] + acc

    def layer(it, carry):
        MT[...] = jnp.zeros(MT.shape, F32)
        Z[...] = jnp.zeros(Z.shape, F32)
        A[...] = jnp.zeros(A.shape, BF)

        def ln_a(s, c):
            r0 = pl.multiple_of(s * L, L)
            XN[pl.ds(r0, L), :] = ln(X[pl.ds(r0, L), :]).astype(BF)
            return c
        lax.fori_loop(0, NSEG, ln_a, 0)

        @pl.when(it == 0)
        def _():
            for n in ("wq", "wk", "wv", "wo"):
                copies[n].wait()

        def seg(s, c):
            def grp(g, c2):
                a_group(s, g)
                return c2
            lax.fori_loop(0, G, grp, 0)
            a_out(s)
            return c
        lax.fori_loop(0, NSEG, seg, 0)

        @pl.when(it == 0)
        def _():
            for n in ("w1", "w2", "w3", "w4"):
                copies[n].wait()

        for c in range(8):
            HB[c, pl.ds(0, 8), :] = jnp.zeros((8, 128), F32)
            HB[c, pl.ds(8 + S, 8), :] = jnp.zeros((8, 128), F32)
        TM = 256

        def b1(t, c):
            r0 = pl.multiple_of(t * TM, TM)
            xn = ln(X[pl.ds(r0, TM), :])
            xnn = ln(xn).astype(BF)
            h = gelu(mm(xnn, w1[...]))
            for cb in range(8):
                HB[cb, pl.ds(pl.multiple_of(r0 + 8, 8), TM), :] = h[:, cb * 128:(cb + 1) * 128]
            XF[pl.ds(r0, TM), :] = xn
            return c
        lax.fori_loop(0, S // TM, b1, 0)

        def b2(t, c):
            r0 = pl.multiple_of(t * TM, TM)
            sh = [-1, -1, 1, 1, -2, -2, 2, 2]
            hsft = jnp.concatenate([HB[cb, pl.ds(r0 + (8 + sh[cb]), TM), :].astype(BF) for cb in range(8)], axis=1)
            x1 = XF[pl.ds(r0, TM), :] + mm(hsft, w2[...])
            x1n = ln(x1).astype(BF)
            u = gelu(mm(x1n, w3[...])).astype(BF)
            y = mm(u, w4[...])
            xnew = X[pl.ds(r0, TM), :] + x1 + y
            X[pl.ds(r0, TM), :] = xnew
            xb[pl.ds(r0, TM), :] = xnew.astype(BF)
            return c
        lax.fori_loop(0, S // TM, b2, 0)
        return carry

    lax.fori_loop(0, 2, layer, 0)
    oc = pltpu.make_async_copy(xb, out_hbm, osem)
    oc.start()
    oc.wait()


@jax.jit
def pallas_interleave_layers__memory_aug_infini_attn__mixer_s_mlp__prompt_kernel(
        A_x, A_wq, A_wk, A_wv, A_wo, A_beta, B_x, B_w1, B_w2, B_w3, B_w4):
    anyspec = pl.BlockSpec(memory_space=pl.ANY)
    V = pltpu.VMEM
    out = pl.pallas_call(
        kernel,
        out_shape=jax.ShapeDtypeStruct((S, D), BF),
        in_specs=[anyspec] * 5 + [pl.BlockSpec(memory_space=pltpu.VMEM)] + [anyspec] * 4,
        out_specs=anyspec,
        scratch_shapes=[
            V((D, D), BF), V((D, D), BF), V((D, D), BF), V((D, D), BF), V((D, D), BF), V((D, D), BF),
            V((D, F), BF), V((F, D), BF),
            V((S, D), BF),
            V((S, D), F32),
            V((S, D), F32),
            V((S, D), BF),
            V((L, 128), BF), V((L, 128), BF), V((L, 128), BF), V((L, 128), BF),
            V((128, L), BF),
            V((G, 128, L), BF),
            V((G, 128, 128), F32),
            V((G, 8, 128), F32),
            V((G, 160, 128), BF),
            V((8, S + 16, 128), F32),
            V((H, 8, 128), F32),
            V((128, 128), F32),
            pltpu.SemaphoreType.DMA((9,)),
            pltpu.SemaphoreType.DMA(()),
        ],
        compiler_params=pltpu.CompilerParams(vmem_limit_bytes=118 * 1024 * 1024),
        name="mykern",
    )(A_x.reshape(S, D), A_wq, A_wk, A_wv, A_wo, A_beta.reshape(1, H), B_w1, B_w2, B_w3, B_w4)
    return out.reshape(1, S, D)
```

```python
import functools
import math

import jax
import jax.numpy as jnp
from jax import lax
import jax.experimental.pallas as pl
import jax.experimental.pallas.tpu as pltpu

S, D, H, DH, NSEG, L, F = 2048, 1024, 32, 32, 4, 512, 3584
G = 8
NF = F // 128
LOG2E = 1.4426950408889634
QSCALE = DH ** -0.5 * LOG2E
NEG = -1e9 * LOG2E
BF = jnp.bfloat16
F32 = jnp.float32
I32 = jnp.int32

NT = (((1,), (1,)), ((), ()))
NN = (((1,), (0,)), ((), ()))
TN = (((0,), (0,)), ((), ()))
TT = (((0,), (1,)), ((), ()))


def mm(a, b, dn=NN):
    return lax.dot_general(a, b, dn, preferred_element_type=F32)


def ld(ref, *idx):
    *lead, rows = idx
    if rows is None:
        v = ref.bitcast(I32)[tuple(lead)]
    else:
        st, n = rows
        st2 = st // 2 if isinstance(st, int) else pl.multiple_of(st // 2, 8)
        v = ref.bitcast(I32)[(*lead, pl.ds(st2, n // 2), slice(None))]
    return pltpu.bitcast(v, BF)


def cat(xs, axis):
    return jnp.concatenate(xs, axis=axis) if len(xs) > 1 else xs[0]


def ln(x):
    m = jnp.mean(x, axis=-1, keepdims=True)
    d = x - m
    v = jnp.mean(d * d, axis=-1, keepdims=True)
    return d * lax.rsqrt(v + 1e-5)


def gelu(x):
    c0 = math.sqrt(2.0 / math.pi)
    u = x * (x * x * (c0 * 0.044715) + c0)
    hx = 0.5 * x
    return hx * jnp.tanh(u) + hx


def phi(t):
    return jnp.where(t > 0, t + 1.0, jnp.exp(t))


def kernel(x_hbm, wq_hbm, wk_hbm, wv_hbm, wo_hbm, beta_ref, w1_hbm, w2_hbm, w3_hbm, w4_hbm,
           out_hbm,
           wq, wk, wv, wo, w1, w2, w3, w4,
           xb, X, XF, XN, MT, Z, A, HB, Gt, bias, SS, MM3, VT3, AM3, OT, sems, osem):
    copies = {}
    xc = pltpu.make_async_copy(x_hbm, xb, sems.at[0])
    xc.start()
    order = [("wq", wq_hbm, wq), ("wk", wk_hbm, wk), ("wv", wv_hbm, wv), ("wo", wo_hbm, wo),
             ("w1", w1_hbm, w1), ("w2", w2_hbm, w2), ("w3", w3_hbm, w3), ("w4", w4_hbm, w4)]
    for i, (n, src, dst) in enumerate(order):
        cs = []
        for c in range(dst.shape[0]):
            cp = pltpu.make_async_copy(src.at[:, pl.ds(c * 128, 128)], dst.at[c], sems.at[i + 1])
            cp.start()
            cs.append(cp)
        copies[n] = cs

    def wait(n):
        for cp in copies[n]:
            cp.wait()

    def full(w, k0=0, k1=None):
        k1 = w.shape[1] if k1 is None else k1
        return cat([ld(w, c, (k0, k1 - k0)) for c in range(w.shape[0])], 1)

    r = lax.broadcasted_iota(I32, (128, 128), 0)
    c = lax.broadcasted_iota(I32, (128, 128), 1)
    bias[...] = jnp.where(r > c, NEG, 0.0).astype(F32)
    blk = (lax.broadcasted_iota(I32, (128, 128), 0) // DH) == (lax.broadcasted_iota(I32, (128, 128), 1) // DH)

    b = beta_ref[...].astype(F32)
    gv = jax.nn.sigmoid(b)
    rr = lax.broadcasted_iota(I32, (H, H), 0)
    cc = lax.broadcasted_iota(I32, (H, H), 1)
    col = jnp.sum(jnp.where(rr == cc, jnp.broadcast_to(gv, (H, H)), 0.0), axis=1, keepdims=True)
    gb = jnp.broadcast_to(col, (H, 128))
    for h in range(H):
        Gt[h] = jnp.broadcast_to(gb[h:h + 1, :], (8, 128))

    SS[...] = jnp.zeros(SS.shape, F32)
    MM3[...] = jnp.zeros(MM3.shape, F32)
    VT3[...] = jnp.zeros(VT3.shape, BF)
    AM3[...] = jnp.zeros(AM3.shape, F32)
    xc.wait()

    def init_x(s, c):
        r0 = pl.multiple_of(s * L, L)
        x = xb[pl.ds(r0, L), :].astype(F32)
        X[pl.ds(r0, L), :] = x
        xn = ln(x).astype(BF)
        for cb in range(8):
            XN[cb, pl.ds(r0, L), :] = xn[:, cb * 128:(cb + 1) * 128]
        return c
    lax.fori_loop(0, NSEG, init_x, 0)

    def xn_tile(r0, n):
        return cat([ld(XN, cb, (r0, n)) for cb in range(8)], 1)

    def a_segment(s):
        r0 = pl.multiple_of(s * L, L)
        st = {}

        def gate(name, v, n):
            st['gate', name + '0'] = v[0:8, 0:128]
            st['gate', name + '1'] = v[n - 8:n, 0:128]

        def proj_k(g, t, gi):
            xn = xn_tile(r0 + 128 * t, 128)
            k = mm(xn, ld(wk, gi, None))
            st['K', g, t] = k.astype(BF)
            gate('prev', k, 128)
            pk = phi(k)
            st['PK', g, t] = pk
            zs = jnp.sum(pk.reshape(16, 8, 128), axis=0)
            st['z', g] = zs if t == 0 else st['z', g] + zs

        def proj_qv(g, t, gi):
            xn = xn_tile(r0 + 128 * t, 128)
            wqv = jnp.concatenate([ld(wq, gi, None), ld(wv, gi, None)], axis=1)
            r = mm(wqv, xn, TT)
            q = r[:128]
            gate('prev', r, 256)
            st['QT', g, t] = q * QSCALE
            st['PQT', g, t] = phi(q)
            st['VT', g, t] = r[128:].astype(BF)

        def qk(g, i, j):
            qt = st['QT', g, i]
            z32 = jnp.zeros((32, 128), F32)
            w = jnp.concatenate([jnp.concatenate([qt[32 * hh:32 * hh + 32] if rr == hh else z32 for rr in range(4)], axis=0)
                                 for hh in range(4)], axis=1).astype(BF)
            s_ = mm(st['K', g, j], w)
            gate('prev', s_, 128)
            if i == j:
                s_ = s_ + jnp.concatenate([bias[...]] * 4, axis=1)
            st['s', g, i, j] = s_
            mx = jnp.max(s_.reshape(16, 8, 512), axis=0)
            st['m', g, i] = mx if j == 0 else jnp.maximum(st['m', g, i], mx)
            if j == i:
                st['m', g, i] = jnp.broadcast_to(jnp.max(st['m', g, i], axis=0, keepdims=True), (8, 512))

        def sm(g, i, j, gt=None):
            m = st['m', g, i] if g != 'c' else MM3[...]
            if gt is not None:
                t = st['gate', gt] * 0.0
                m = m + jnp.concatenate([t] * 4, axis=1)
            s_ = st.pop(('s', g, i, j)) if g != 'c' else SS[j]
            ps = []
            for c in range(8):
                e0 = jnp.exp2(s_[16 * c:16 * c + 8] - m)
                e1 = jnp.exp2(s_[16 * c + 8:16 * c + 16] - m)
                ee = e0 + e1
                st['l', g, i] = ee if (j == 0 and c == 0) else st['l', g, i] + ee
                ps.append(e0); ps.append(e1)
            st['p', g, i, j] = jnp.concatenate(ps, axis=0)

        def pv(g, i, j):
            pb = st.pop(('p', g, i, j))
            for hh in range(4):
                vt = st['VT', g, j][32 * hh:32 * hh + 32] if g != 'c' else ld(VT3, j, (32 * hh, 32))
                ot = mm(vt, pb[:, 128 * hh:128 * (hh + 1)].astype(BF))
                st['o', g, i, hh] = ot if j == 0 else st['o', g, i, hh] + ot

        def memrd(g, gi):
            pq = cat([st['PQT', g, t] for t in range(4)], 1).astype(BF)
            mem = mm(ld(A, gi, None), pq)
            gate('prev', mem, 160)
            for hh in range(4):
                g1 = Gt[gi * 4 + hh][0:1, :]
                den = mem[40 * hh + 32:40 * hh + 33, :] + 1e-6
                wm = g1[:, 0:1] / den
                st['AM', g, hh] = mem[40 * hh:40 * hh + 32, :] * wm

        def fin(g, i, gi=None):
            gi = g if gi is None else gi
            l = jnp.sum(st['l', g, i], axis=0, keepdims=True)
            os_ = []
            for hh in range(4):
                g1 = Gt[gi * 4 + hh][0:1, :]
                wd = (1.0 - g1) / l[:, 128 * hh:128 * (hh + 1)]
                am = st['AM', g, hh][:, 128 * i:128 * (i + 1)] if g != 'c' else AM3[pl.ds(32 * hh, 32), :]
                os_.append(st['o', g, i, hh] * wd + am)
            OT[gi, i] = jnp.concatenate(os_, axis=0).astype(BF)

        def save_tail(g):
            for j in range(4):
                SS[j] = st.pop(('s', g, 3, j))
                VT3[j] = st['VT', g, j]
            MM3[...] = st['m', g, 3]
            for hh in range(4):
                AM3[pl.ds(32 * hh, 32), :] = st['AM', g, hh][:, 384:512]

        def upd(g, gi):
            pk = cat([st['PK', g, t] for t in range(4)], 0).astype(BF)
            d = mm(cat([st['VT', g, t] for t in range(4)], 1), pk)
            gate('prev', d, 128)
            mt = MT[gi] + jnp.where(blk, d, 0.0)
            MT[gi] = mt
            z = Z[gi] + jnp.broadcast_to(jnp.sum(st['z', g], axis=0, keepdims=True), (8, 128))
            Z[gi] = z
            lh = lax.broadcasted_iota(I32, (8, 128), 1) // DH
            parts = []
            for hh in range(4):
                parts.append(mt[32 * hh:32 * hh + 32, :])
                parts.append(jnp.where(lh == hh, z, 0.0))
            A[gi] = jnp.concatenate(parts, axis=0).astype(BF)

        def aout(i, part=None):
            rows = pl.ds(r0 + 128 * i, 128)
            ot = cat([ld(OT, g, i, None) for g in range(G)], 0)
            acc = mm(ot, full(wo), TN)
            gate('prev', acc, 128)
            x = X[rows, :] + acc
            xn = ln(x)
            X[rows, :] = x
            XF[rows, :] = xn
            st['xnn', i] = ln(xn).astype(BF)

        def hproj(i):
            h = gelu(mm(st['xnn', i], full(w1)))
            for cb in range(8):
                HB[cb, pl.ds(pl.multiple_of(r0 + 128 * i + 8, 8), 128), :] = h[:, cb * 128:(cb + 1) * 128]

        def group(g, gi, p, pi):
            proj_k(g, 0, gi)
            sm(p, 3, 0)
            sm(p, 3, 1, 'prev0'); pv(p, 3, 0)
            proj_qv(g, 0, gi)
            sm(p, 3, 2, 'prev1'); pv(p, 3, 1)
            qk(g, 0, 0)
            proj_k(g, 1, gi)
            sm(p, 3, 3, 'prev0'); pv(p, 3, 2)
            proj_qv(g, 1, gi)
            sm(g, 0, 0, 'prev0')
            pv(p, 3, 3); fin(p, 3, pi)
            qk(g, 1, 0)
            qk(g, 1, 1)
            sm(g, 1, 0)
            pv(g, 0, 0)
            proj_k(g, 2, gi)
            pv(g, 1, 0)
            proj_qv(g, 2, gi)
            sm(g, 1, 1, 'prev0')
            qk(g, 2, 0)
            pv(g, 1, 1)
            qk(g, 2, 1)
            qk(g, 2, 2)
            sm(g, 2, 0)
            proj_k(g, 3, gi)
            pv(g, 2, 0)
            proj_qv(g, 3, gi)
            sm(g, 2, 1, 'prev0')
            memrd(g, gi)
            pv(g, 2, 1)
            qk(g, 3, 0)
            sm(g, 2, 2, 'prev0')
            qk(g, 3, 1)
            qk(g, 3, 2)
            pv(g, 2, 2)
            fin(g, 0, gi); fin(g, 1, gi); fin(g, 2, gi)
            qk(g, 3, 3)
            upd(g, gi)

        NG = 4

        def gl(k, c):
            g0 = k * NG
            for g in range(NG):
                if g == 0:
                    group(g, g0, 'c', (g0 + G - 1) % G)
                else:
                    group(g, g0 + g, g - 1, g0 + g - 1)
            save_tail(NG - 1)
            return c
        lax.fori_loop(0, G // NG, gl, 0)
        st.clear()
        p = 'c'
        aout(0)
        sm(p, 3, 0)
        sm(p, 3, 1, 'prev0'); pv(p, 3, 0)
        aout(1)
        sm(p, 3, 2, 'prev0'); pv(p, 3, 1)
        hproj(0)
        sm(p, 3, 3, 'prev1'); pv(p, 3, 2)
        aout(2)
        pv(p, 3, 3); fin(p, 3, G - 1)
        hproj(1)
        aout(3)
        hproj(2)
        hproj(3)

    def layer(it, carry):
        MT[...] = jnp.zeros(MT.shape, F32)
        Z[...] = jnp.zeros(Z.shape, F32)
        A[...] = jnp.zeros(A.shape, BF)

        @pl.when(it == 0)
        def _():
            for n in ("wq", "wk", "wv", "wo", "w1"):
                wait(n)

        def seg(s, c):
            a_segment(s)
            return c
        lax.fori_loop(0, NSEG, seg, 0)

        @pl.when(it == 0)
        def _():
            for n in ("w2", "w3", "w4"):
                wait(n)

        TM = 256

        def b2(t, c):
            r0 = pl.multiple_of(t * TM, TM)
            sh = [-1, -1, 1, 1, -2, -2, 2, 2]
            hsft = jnp.concatenate([HB[cb, pl.ds(r0 + (8 + sh[cb]), TM), :].astype(BF) for cb in range(8)], axis=1)
            x1 = XF[pl.ds(r0, TM), :] + mm(hsft, full(w2))
            x1n = ln(x1).astype(BF)
            u = gelu(mm(x1n, full(w3))).astype(BF)
            y = mm(u, full(w4))
            xnew = X[pl.ds(r0, TM), :] + x1 + y
            X[pl.ds(r0, TM), :] = xnew
            xb[pl.ds(r0, TM), :] = xnew.astype(BF)
            xn = ln(xnew).astype(BF)
            for cb in range(8):
                XN[cb, pl.ds(r0, TM), :] = xn[:, cb * 128:(cb + 1) * 128]
            return c
        lax.fori_loop(0, S // TM, b2, 0)
        return carry

    for c in range(8):
        HB[c, pl.ds(0, 8), :] = jnp.zeros((8, 128), F32)
        HB[c, pl.ds(8 + S, 8), :] = jnp.zeros((8, 128), F32)
    lax.fori_loop(0, 2, layer, 0)
    oc = pltpu.make_async_copy(xb, out_hbm, osem)
    oc.start()
    oc.wait()


@jax.jit
def pallas_interleave_layers__memory_aug_infini_attn__mixer_s_mlp__prompt_kernel(
        A_x, A_wq, A_wk, A_wv, A_wo, A_beta, B_x, B_w1, B_w2, B_w3, B_w4):
    anyspec = pl.BlockSpec(memory_space=pl.ANY)
    V = pltpu.VMEM
    wsq = V((G, D, 128), BF)
    out = pl.pallas_call(
        kernel,
        out_shape=jax.ShapeDtypeStruct((S, D), BF),
        in_specs=[anyspec] * 5 + [pl.BlockSpec(memory_space=pltpu.VMEM)] + [anyspec] * 4,
        out_specs=anyspec,
        scratch_shapes=[
            wsq, wsq, wsq, wsq, wsq, wsq,
            V((NF, D, 128), BF), V((G, F, 128), BF),
            V((S, D), BF),
            V((S, D), F32),
            V((S, D), F32),
            V((G, S, 128), BF),
            V((G, 128, 128), F32),
            V((G, 8, 128), F32),
            V((G, 160, 128), BF),
            V((8, S + 16, 128), F32),
            V((H, 8, 128), F32),
            V((128, 128), F32),
            V((4, 128, 512), F32),
            V((8, 512), F32),
            V((4, 128, 128), BF),
            V((128, 128), F32),
            V((G, 4, 128, 128), BF),
            pltpu.SemaphoreType.DMA((9,)),
            pltpu.SemaphoreType.DMA(()),
        ],
        compiler_params=pltpu.CompilerParams(vmem_limit_bytes=118 * 1024 * 1024),
        name="mykern",
    )(A_x.reshape(S, D), A_wq, A_wk, A_wv, A_wo, A_beta.reshape(1, H), B_w1, B_w2, B_w3, B_w4)
    return out.reshape(1, S, D)
```

```python
import functools
import math

import jax
import jax.numpy as jnp
from jax import lax
import jax.experimental.pallas as pl
import jax.experimental.pallas.tpu as pltpu

S, D, H, DH, NSEG, L, F = 2048, 1024, 32, 32, 4, 512, 3584
G = 8
NG = 4
NF = F // 128
TM = 256
LOG2E = 1.4426950408889634
QSCALE = DH ** -0.5 * LOG2E
NEG = -1e9 * LOG2E
BF = jnp.bfloat16
F32 = jnp.float32
I32 = jnp.int32

NN = (((1,), (0,)), ((), ()))
TN = (((0,), (0,)), ((), ()))
TT = (((0,), (1,)), ((), ()))


def mm(a, b, dn=NN):
    return lax.dot_general(a, b, dn, preferred_element_type=F32)


def ld(ref, *idx):
    *lead, rows = idx
    if rows is None:
        v = ref.bitcast(I32)[tuple(lead)]
    else:
        st, n = rows
        st2 = st // 2 if isinstance(st, int) else pl.multiple_of(st // 2, 8)
        v = ref.bitcast(I32)[(*lead, pl.ds(st2, n // 2), slice(None))]
    return pltpu.bitcast(v, BF)


def cat(xs, axis):
    return jnp.concatenate(xs, axis=axis) if len(xs) > 1 else xs[0]


def ln(x):
    m = jnp.mean(x, axis=-1, keepdims=True)
    d = x - m
    v = jnp.mean(d * d, axis=-1, keepdims=True)
    return d * lax.rsqrt(v + 1e-5)


def ln2(x):
    m = jnp.mean(x, axis=-1, keepdims=True)
    d = x - m
    v = jnp.mean(d * d, axis=-1, keepdims=True)
    r = lax.rsqrt(v + 1e-5)
    r2 = lax.rsqrt(v * r * r + 1e-5)
    return d * r, d * (r * r2)


def gelu(x):
    c0 = math.sqrt(2.0 / math.pi)
    u = x * (x * x * (c0 * 0.044715) + c0)
    hx = 0.5 * x
    return hx * jnp.tanh(u) + hx


def phi(t):
    return jnp.where(t > 0, t + 1.0, jnp.exp(t))


def tok(x, gate):
    if gate is None:
        return x
    t = gate * 0.0
    if x.shape[0] != 8:
        t = cat([t] * (x.shape[0] // 8), 0)
    return x + cat([t] * (x.shape[1] // 128), 1)


def inject(v, toks):
    if not toks:
        return v
    d = dict(toks)
    top = cat([v[0:8, 128 * c:128 * (c + 1)] + d[c] * 0.0 if c in d else v[0:8, 128 * c:128 * (c + 1)]
               for c in range(v.shape[1] // 128)], 1)
    return cat([top, v[8:]], 0) if v.shape[0] > 8 else top


def kernel(x_hbm, wq_hbm, wk_hbm, wv_hbm, wo_hbm, beta_ref, w1_hbm, w2_hbm, w3_hbm, w4_hbm,
           out_hbm,
           wq, wk, wv, wo, w1, w2, w3, w4,
           xb, X, XF, XN, MT, Z, A, HB, Gt, bias, SS, MM3, VT3, AM3, OT,
           sx, sq, sk, sv, sw, so):
    def x_copy(s):
        return pltpu.make_async_copy(x_hbm.at[pl.ds(s * L, L), :], xb.at[pl.ds(s * L, L), :], sx.at[s])

    def qkv_copies(g):
        c0 = g * 128 if isinstance(g, int) else pl.multiple_of(g * 128, 128)
        return [pltpu.make_async_copy(src.at[:, pl.ds(c0, 128)], dst.at[g], sem.at[g])
                for src, dst, sem in ((wk_hbm, wk, sk), (wq_hbm, wq, sq), (wv_hbm, wv, sv))]

    def w_copies(i, src, dst):
        return [pltpu.make_async_copy(src.at[:, pl.ds(c * 128, 128)], dst.at[c], sw.at[i]) for c in range(dst.shape[0])]

    def out_copy(t):
        r0 = t * TM if isinstance(t, int) else pl.multiple_of(t * TM, TM)
        return pltpu.make_async_copy(xb.at[pl.ds(r0, TM), :], out_hbm.at[pl.ds(r0, TM), :], so.at[t])

    wl = {"wo": (0, wo_hbm, wo), "w1": (1, w1_hbm, w1), "w2": (2, w2_hbm, w2), "w3": (3, w3_hbm, w3), "w4": (4, w4_hbm, w4)}
    x_copy(0).start()
    for g in range(NG):
        for cp in qkv_copies(g):
            cp.start()

    def start_batch2():
        for g in range(NG, G):
            for cp in qkv_copies(g):
                cp.start()
        for n in ("wo", "w1"):
            for cp in w_copies(*wl[n]):
                cp.start()
        x_copy(1).start()

    def start_batch3():
        for s in range(2, NSEG):
            x_copy(s).start()
        for n in ("w2", "w3", "w4"):
            for cp in w_copies(*wl[n]):
                cp.start()

    def wait(n):
        for cp in w_copies(*wl[n]):
            cp.wait()

    def full(w, k0=0, k1=None, cols=None):
        k1 = w.shape[1] if k1 is None else k1
        cols = range(w.shape[0]) if cols is None else cols
        return cat([ld(w, c, (k0, k1 - k0)) for c in cols], 1)

    r = lax.broadcasted_iota(I32, (128, 128), 0)
    c = lax.broadcasted_iota(I32, (128, 128), 1)
    bias[...] = jnp.where(r > c, NEG, 0.0).astype(F32)
    blk = (lax.broadcasted_iota(I32, (128, 128), 0) // DH) == (lax.broadcasted_iota(I32, (128, 128), 1) // DH)

    b = beta_ref[...].astype(F32)
    gv = jax.nn.sigmoid(b)
    rr = lax.broadcasted_iota(I32, (H, H), 0)
    cc = lax.broadcasted_iota(I32, (H, H), 1)
    col = jnp.sum(jnp.where(rr == cc, jnp.broadcast_to(gv, (H, H)), 0.0), axis=1, keepdims=True)
    gb = jnp.broadcast_to(col, (H, 128))
    for h in range(H):
        Gt[h] = jnp.broadcast_to(gb[h:h + 1, :], (8, 128))
    SS[...] = jnp.zeros(SS.shape, F32)
    MM3[...] = jnp.zeros(MM3.shape, F32)
    VT3[...] = jnp.zeros(VT3.shape, BF)
    AM3[...] = jnp.zeros(AM3.shape, F32)
    for c in range(8):
        HB[c, pl.ds(0, 8), :] = jnp.zeros((8, 128), F32)
        HB[c, pl.ds(8 + S, 8), :] = jnp.zeros((8, 128), F32)

    def ln_a(r0, n, gate=None):
        xf = ln(tok(xb[pl.ds(r0, n), :].astype(F32), gate))
        xn = xf.astype(BF)
        for cb in range(8):
            XN[cb, pl.ds(r0, n), :] = xn[:, cb * 128:(cb + 1) * 128]
        t = jnp.sum(xf.reshape(n // 8, 8, D), axis=0)
        return functools.reduce(jnp.add, [t[:, 128 * cb:128 * (cb + 1)] for cb in range(8)])

    x_copy(0).wait()

    def ln0(t, c):
        ln_a(pl.multiple_of(t * 128, 128), 128)
        return c
    lax.fori_loop(0, L // 128, ln0, 0)

    def xn_tile(r0, n):
        return cat([ld(XN, cb, (r0, n)) for cb in range(8)], 1)

    def a_segment(it, s):
        r0 = pl.multiple_of(s * L, L)
        first = jnp.logical_and(it == 0, s == 0)
        st = {}

        def gate(name, v, n):
            st['gate', name + '0'] = v[0:8, 0:128]
            st['gate', name + '1'] = v[n - 8:n, 0:128]

        def proj_k(g, t, gi):
            xn = xn_tile(r0 + 128 * t, 128)
            k = mm(xn, ld(wk, gi, None))
            st['K', g, t] = k.astype(BF)
            gate('prev', k, 128)
            pk = phi(k)
            st['PK', g, t] = pk
            zs = jnp.sum(pk.reshape(16, 8, 128), axis=0)
            st['z', g] = zs if t == 0 else st['z', g] + zs

        def proj_qv(g, t, gi):
            xn = xn_tile(r0 + 128 * t, 128)
            wqv = jnp.concatenate([ld(wq, gi, None), ld(wv, gi, None)], axis=1)
            r = mm(wqv, xn, TT)
            q = r[:128]
            gate('prev', r, 256)
            st['QT', g, t] = q * QSCALE
            st['PQT', g, t] = phi(q)
            st['VT', g, t] = r[128:].astype(BF)

        def qk(g, i, j):
            qt = st['QT', g, i]
            z32 = jnp.zeros((32, 128), F32)
            w = jnp.concatenate([jnp.concatenate([qt[32 * hh:32 * hh + 32] if rr == hh else z32 for rr in range(4)], axis=0)
                                 for hh in range(4)], axis=1).astype(BF)
            s_ = mm(st['K', g, j], w)
            gate('prev', s_, 128)
            if i == j:
                s_ = s_ + jnp.concatenate([bias[...]] * 4, axis=1)
            st['s', g, i, j] = s_
            mx = jnp.max(s_.reshape(16, 8, 512), axis=0)
            st['m', g, i] = mx if j == 0 else jnp.maximum(st['m', g, i], mx)
            if j == i:
                st['m', g, i] = jnp.broadcast_to(jnp.max(st['m', g, i], axis=0, keepdims=True), (8, 512))

        def sm(g, i, j, gt=None):
            m = st['m', g, i] if g != 'c' else MM3[...]
            m = tok(m, st['gate', gt] if gt else None)
            s_ = st.pop(('s', g, i, j)) if g != 'c' else SS[j]
            ps = []
            for c in range(8):
                e0 = jnp.exp2(s_[16 * c:16 * c + 8] - m)
                e1 = jnp.exp2(s_[16 * c + 8:16 * c + 16] - m)
                ee = e0 + e1
                st['l', g, i] = ee if (j == 0 and c == 0) else st['l', g, i] + ee
                ps.append(e0); ps.append(e1)
            st['p', g, i, j] = jnp.concatenate(ps, axis=0)

        def pv(g, i, j):
            pb = st.pop(('p', g, i, j))
            for hh in range(4):
                vt = st['VT', g, j][32 * hh:32 * hh + 32] if g != 'c' else ld(VT3, j, (32 * hh, 32))
                ot = mm(vt, pb[:, 128 * hh:128 * (hh + 1)].astype(BF))
                st['o', g, i, hh] = ot if j == 0 else st['o', g, i, hh] + ot

        def memrd(g, gi):
            pq = cat([st['PQT', g, t] for t in range(4)], 1).astype(BF)
            mem = mm(ld(A, gi, None), pq)
            gate('prev', mem, 160)
            for hh in range(4):
                g1 = Gt[gi * 4 + hh][0:1, :]
                den = mem[40 * hh + 32:40 * hh + 33, :] + 1e-6
                wm = g1[:, 0:1] / den
                st['AM', g, hh] = mem[40 * hh:40 * hh + 32, :] * wm

        def fin(g, i, gi):
            l = jnp.sum(st['l', g, i], axis=0, keepdims=True)
            os_ = []
            for hh in range(4):
                g1 = Gt[gi * 4 + hh][0:1, :]
                wd = (1.0 - g1) / l[:, 128 * hh:128 * (hh + 1)]
                am = st['AM', g, hh][:, 128 * i:128 * (i + 1)] if g != 'c' else AM3[pl.ds(32 * hh, 32), :]
                os_.append(st['o', g, i, hh] * wd + am)
            OT[gi, i] = jnp.concatenate(os_, axis=0).astype(BF)

        def save_tail(g):
            for j in range(4):
                SS[j] = st.pop(('s', g, 3, j))
                VT3[j] = st['VT', g, j]
            MM3[...] = st['m', g, 3]
            for hh in range(4):
                AM3[pl.ds(32 * hh, 32), :] = st['AM', g, hh][:, 384:512]

        def upd(g, gi):
            pk = cat([st['PK', g, t] for t in range(4)], 0).astype(BF)
            d = mm(cat([st['VT', g, t] for t in range(4)], 1), pk)
            gate('prev', d, 128)
            mt = MT[gi] + jnp.where(blk, d, 0.0)
            MT[gi] = mt
            z = Z[gi] + jnp.broadcast_to(jnp.sum(st['z', g], axis=0, keepdims=True), (8, 128))
            Z[gi] = z
            lh = lax.broadcasted_iota(I32, (8, 128), 1) // DH
            parts = []
            for hh in range(4):
                parts.append(mt[32 * hh:32 * hh + 32, :])
                parts.append(jnp.where(lh == hh, z, 0.0))
            A[gi] = jnp.concatenate(parts, axis=0).astype(BF)

        def group(g, gi, p, pi):
            proj_k(g, 0, gi)
            sm(p, 3, 0)
            sm(p, 3, 1, 'prev0'); pv(p, 3, 0)
            proj_qv(g, 0, gi)
            sm(p, 3, 2, 'prev1'); pv(p, 3, 1)
            qk(g, 0, 0)
            proj_k(g, 1, gi)
            sm(p, 3, 3, 'prev0'); pv(p, 3, 2)
            proj_qv(g, 1, gi)
            sm(g, 0, 0, 'prev0')
            pv(p, 3, 3); fin(p, 3, pi)
            qk(g, 1, 0)
            qk(g, 1, 1)
            sm(g, 1, 0)
            pv(g, 0, 0)
            proj_k(g, 2, gi)
            pv(g, 1, 0)
            proj_qv(g, 2, gi)
            sm(g, 1, 1, 'prev0')
            qk(g, 2, 0)
            pv(g, 1, 1)
            qk(g, 2, 1)
            qk(g, 2, 2)
            sm(g, 2, 0)
            proj_k(g, 3, gi)
            pv(g, 2, 0)
            proj_qv(g, 3, gi)
            sm(g, 2, 1, 'prev0')
            memrd(g, gi)
            pv(g, 2, 1)
            qk(g, 3, 0)
            sm(g, 2, 2, 'prev0')
            qk(g, 3, 1)
            qk(g, 3, 2)
            pv(g, 2, 2)
            fin(g, 0, gi); fin(g, 1, gi); fin(g, 2, gi)
            qk(g, 3, 3)
            upd(g, gi)

        def gl(k, c):
            g0 = k * NG

            @pl.when(first)
            def _():
                for g in range(NG):
                    for cp in qkv_copies(g0 + g):
                        cp.wait()

                @pl.when(k == 0)
                def _():
                    start_batch2()

            for g in range(NG):
                if g == 0:
                    group(g, g0, 'c', (g0 + G - 1) % G)
                else:
                    group(g, g0 + g, g - 1, g0 + g - 1)
            save_tail(NG - 1)
            return c
        lax.fori_loop(0, G // NG, gl, 0)
        st.clear()

        @pl.when(first)
        def _():
            wait("wo")
            wait("w1")
            start_batch3()

        sn = jnp.minimum(s + 1, NSEG - 1)

        @pl.when(jnp.logical_and(it == 0, s < NSEG - 1))
        def _():
            x_copy(sn).wait()

        pend = []

        def drain(acc):
            for e in pend:
                e[0] -= 1
            ready = [e[1] for e in pend if e[0] <= 0]
            pend[:] = [e for e in pend if e[0] > 0]
            for t in ready:
                acc = inject(acc, [(0, t)])
            return acc

        def aout(i, fill=()):
            rows = pl.ds(r0 + 128 * i, 128)
            ot = cat([ld(OT, g, i, None) for g in range(G)], 0)
            xs = []
            for n in range(8):
                acc = mm(ot, ld(wo, n, None), TN)
                acc = drain(acc)
                if n < len(fill) and fill[n] is not None:
                    fill[n](acc[0:8])
                xs.append(acc)
            x = xb[rows, :].astype(F32) + cat(xs, 1)
            X[rows, :] = x
            st['x', i] = x

        def lnb(i, c):
            def f(gate):
                rows = pl.ds(r0 + 128 * i + 32 * c, 32)
                xn, xnn = ln2(tok(st['x', i][32 * c:32 * c + 32], gate))
                XF[rows, :] = xn
                st['xnn', i, c] = xnn
            return f

        def lna(c):
            def f(gate):
                pend.append([2, ln_a(pl.multiple_of(sn * L + 64 * c, 64), 64, gate)])
            return f

        def hproj(i, fill=()):
            xnn = cat([st['xnn', i, c] for c in range(4)], 0).astype(BF)
            for n in range(8):
                acc = mm(xnn, ld(w1, n, None))
                acc = drain(acc)
                if n < len(fill) and fill[n] is not None:
                    fill[n](acc[0:8])
                HB[n, pl.ds(pl.multiple_of(r0 + 128 * i + 8, 8), 128), :] = gelu(acc)

        p = 'c'

        def psm(j):
            def f(gate):
                st['gate', 'x'] = gate
                sm(p, 3, j, 'x')
            return f

        def lnbs(i):
            return [lnb(i, 0), lnb(i, 1), lnb(i, 2), None, lnb(i, 3)]

        aout(0, [psm(0), lna(0), None, psm(1), lna(1), None, psm(2), lna(2)])
        pv(p, 3, 0); pv(p, 3, 1)
        aout(1, lnbs(0))
        pv(p, 3, 2)
        hproj(0, lnbs(1))
        aout(2, [psm(3), lna(3), None, lna(4), None, lna(5)])
        pv(p, 3, 3); fin(p, 3, G - 1)
        hproj(1, lnbs(2))
        aout(3, [lna(6), None, None, lna(7)])
        hproj(2, lnbs(3))
        hproj(3)

    def layer(it, carry):
        MT[...] = jnp.zeros(MT.shape, F32)
        Z[...] = jnp.zeros(Z.shape, F32)
        A[...] = jnp.zeros(A.shape, BF)

        def seg(s, c):
            a_segment(it, s)
            return c
        lax.fori_loop(0, NSEG, seg, 0)

        @pl.when(it == 0)
        def _():
            for n in ("w2", "w3", "w4"):
                wait(n)

        def b2(t, c):
            r0 = pl.multiple_of(t * TM, TM)
            sh = [-1, -1, 1, 1, -2, -2, 2, 2]
            HM = TM // 2
            x1 = []
            u = []
            for a in range(2):
                ra = r0 + a * HM
                hsft = jnp.concatenate([HB[cb, pl.ds(ra + (8 + sh[cb]), HM), :].astype(BF) for cb in range(8)], axis=1)
                x1.append(XF[pl.ds(ra, HM), :] + mm(hsft, full(w2)))
            tp = (t + (S // TM) - 2) % (S // TM)
            x1n = cat([ln(x1[a]) for a in range(2)], 0).astype(BF)
            pre = mm(x1n, full(w3))
            toks = []
            for cch in range(4):
                g = pre[0:8, 128 * (6 * cch):128 * (6 * cch + 1)]
                toks.append((6 * cch + 5, ln_a(pl.multiple_of(tp * TM + cch * 64, 64), 64, g)))
            u = gelu(inject(pre, toks)).astype(BF)
            y = mm(u, full(w4))
            xnew = X[pl.ds(r0, TM), :] + cat(x1, 0) + y
            xb[pl.ds(r0, TM), :] = xnew.astype(BF)

            @pl.when(it == 1)
            def _():
                out_copy(t).start()
            return c
        lax.fori_loop(0, S // TM, b2, 0)
        return carry

    lax.fori_loop(0, 2, layer, 0)
    for t in range(S // TM):
        out_copy(t).wait()


@jax.jit
def pallas_interleave_layers__memory_aug_infini_attn__mixer_s_mlp__prompt_kernel(
        A_x, A_wq, A_wk, A_wv, A_wo, A_beta, B_x, B_w1, B_w2, B_w3, B_w4):
    anyspec = pl.BlockSpec(memory_space=pl.ANY)
    V = pltpu.VMEM
    wsq = V((G, D, 128), BF)
    dma = pltpu.SemaphoreType.DMA
    out = pl.pallas_call(
        kernel,
        out_shape=jax.ShapeDtypeStruct((S, D), BF),
        in_specs=[anyspec] * 5 + [pl.BlockSpec(memory_space=pltpu.VMEM)] + [anyspec] * 4,
        out_specs=anyspec,
        scratch_shapes=[
            wsq, wsq, wsq, wsq, wsq, wsq,
            V((NF, D, 128), BF), V((G, F, 128), BF),
            V((S, D), BF),
            V((S, D), F32),
            V((S, D), F32),
            V((G, S, 128), BF),
            V((G, 128, 128), F32),
            V((G, 8, 128), F32),
            V((G, 160, 128), BF),
            V((8, S + 16, 128), F32),
            V((H, 8, 128), F32),
            V((128, 128), F32),
            V((4, 128, 512), F32),
            V((8, 512), F32),
            V((4, 128, 128), BF),
            V((128, 128), F32),
            V((G, 4, 128, 128), BF),
            dma((NSEG,)), dma((G,)), dma((G,)), dma((G,)), dma((5,)), dma((S // TM,)),
        ],
        compiler_params=pltpu.CompilerParams(vmem_limit_bytes=118 * 1024 * 1024),
        name="mykern",
    )(A_x.reshape(S, D), A_wq, A_wk, A_wv, A_wo, A_beta.reshape(1, H), B_w1, B_w2, B_w3, B_w4)
    return out.reshape(1, S, D)
```

```python
import functools
import math

import jax
import jax.numpy as jnp
from jax import lax
import jax.experimental.pallas as pl
import jax.experimental.pallas.tpu as pltpu

S, D, H, DH, NSEG, L, F = 2048, 1024, 32, 32, 4, 512, 3584
G = 8
NG = 4
NF = F // 128
TM = 256
LOG2E = 1.4426950408889634
QSCALE = DH ** -0.5 * LOG2E
NEG = -1e9 * LOG2E
BF = jnp.bfloat16
F32 = jnp.float32
I32 = jnp.int32

NN = (((1,), (0,)), ((), ()))
TN = (((0,), (0,)), ((), ()))
TT = (((0,), (1,)), ((), ()))


def mm(a, b, dn=NN):
    return lax.dot_general(a, b, dn, preferred_element_type=F32)


def ld(ref, *idx):
    *lead, rows = idx
    if rows is None:
        v = ref.bitcast(I32)[tuple(lead)]
    else:
        st, n = rows
        st2 = st // 2 if isinstance(st, int) else pl.multiple_of(st // 2, 8)
        v = ref.bitcast(I32)[(*lead, pl.ds(st2, n // 2), slice(None))]
    return pltpu.bitcast(v, BF)


def cat(xs, axis):
    return jnp.concatenate(xs, axis=axis) if len(xs) > 1 else xs[0]


def ln(x):
    m = jnp.mean(x, axis=-1, keepdims=True)
    d = x - m
    v = jnp.mean(d * d, axis=-1, keepdims=True)
    return d * lax.rsqrt(v + 1e-5)


def ln2(x):
    m = jnp.mean(x, axis=-1, keepdims=True)
    d = x - m
    v = jnp.mean(d * d, axis=-1, keepdims=True)
    r = lax.rsqrt(v + 1e-5)
    r2 = lax.rsqrt(v * r * r + 1e-5)
    return d * r, d * (r * r2)


def gelu(x):
    c0 = math.sqrt(2.0 / math.pi)
    u = x * (x * x * (c0 * 0.044715) + c0)
    hx = 0.5 * x
    return hx * jnp.tanh(u) + hx


def phi(t):
    return jnp.where(t > 0, t + 1.0, jnp.exp(t))


def tok(x, gate):
    if gate is None:
        return x
    t = gate * 0.0
    if x.shape[0] != 8:
        t = cat([t] * (x.shape[0] // 8), 0)
    return x + cat([t] * (x.shape[1] // 128), 1)


def tok1(x, gate):
    if gate is None:
        return x
    return cat([tok(x[:, 0:128], gate), x[:, 128:]], 1)


def inject(v, toks):
    if not toks:
        return v
    d = dict(toks)
    top = cat([v[0:8, 128 * c:128 * (c + 1)] + d[c] * 0.0 if c in d else v[0:8, 128 * c:128 * (c + 1)]
               for c in range(v.shape[1] // 128)], 1)
    return cat([top, v[8:]], 0) if v.shape[0] > 8 else top


def kernel(x_hbm, wq_hbm, wk_hbm, wv_hbm, wo_hbm, beta_ref, w1_hbm, w2_hbm, w3_hbm, w4_hbm,
           out_hbm,
           wq, wk, wv, wo, w1, w2, w3, w4,
           xb, X, XF, XN, MT, Z, A, HB, Gt, bias, SS, MM3, VT3, AM3, OT,
           sx, sq, sk, sv, sw, so):
    def x_copy(s):
        return pltpu.make_async_copy(x_hbm.at[pl.ds(s * L, L), :], xb.at[pl.ds(s * L, L), :], sx.at[s])

    def qkv_copies(g):
        c0 = g * 128 if isinstance(g, int) else pl.multiple_of(g * 128, 128)
        return [pltpu.make_async_copy(src.at[:, pl.ds(c0, 128)], dst.at[g], sem.at[g])
                for src, dst, sem in ((wk_hbm, wk, sk), (wq_hbm, wq, sq), (wv_hbm, wv, sv))]

    def w_copies(i, src, dst):
        return [pltpu.make_async_copy(src.at[:, pl.ds(c * 128, 128)], dst.at[c], sw.at[i]) for c in range(dst.shape[0])]

    def out_copy(t):
        r0 = t * TM if isinstance(t, int) else pl.multiple_of(t * TM, TM)
        return pltpu.make_async_copy(xb.at[pl.ds(r0, TM), :], out_hbm.at[pl.ds(r0, TM), :], so.at[t])

    wl = {"wo": (0, wo_hbm, wo), "w1": (1, w1_hbm, w1), "w2": (2, w2_hbm, w2), "w3": (3, w3_hbm, w3), "w4": (4, w4_hbm, w4)}
    x_copy(0).start()
    for g in range(NG):
        for cp in qkv_copies(g):
            cp.start()

    def start_batch2():
        for g in range(NG, G):
            for cp in qkv_copies(g):
                cp.start()
        for n in ("wo", "w1"):
            for cp in w_copies(*wl[n]):
                cp.start()
        x_copy(1).start()

    def start_batch3():
        for s in range(2, NSEG):
            x_copy(s).start()
        for n in ("w2", "w3", "w4"):
            for cp in w_copies(*wl[n]):
                cp.start()

    def wait(n):
        for cp in w_copies(*wl[n]):
            cp.wait()

    def full(w, k0=0, k1=None, cols=None):
        k1 = w.shape[1] if k1 is None else k1
        cols = range(w.shape[0]) if cols is None else cols
        return cat([ld(w, c, (k0, k1 - k0)) for c in cols], 1)

    r = lax.broadcasted_iota(I32, (128, 128), 0)
    c = lax.broadcasted_iota(I32, (128, 128), 1)
    bias[...] = jnp.where(r > c, NEG, 0.0).astype(F32)
    blk = (lax.broadcasted_iota(I32, (128, 128), 0) // DH) == (lax.broadcasted_iota(I32, (128, 128), 1) // DH)

    b = beta_ref[...].astype(F32)
    gv = jax.nn.sigmoid(b)
    rr = lax.broadcasted_iota(I32, (H, H), 0)
    cc = lax.broadcasted_iota(I32, (H, H), 1)
    col = jnp.sum(jnp.where(rr == cc, jnp.broadcast_to(gv, (H, H)), 0.0), axis=1, keepdims=True)
    gb = jnp.broadcast_to(col, (H, 128))
    for h in range(H):
        Gt[h] = jnp.broadcast_to(gb[h:h + 1, :], (8, 128))
    SS[...] = jnp.zeros(SS.shape, F32)
    MM3[...] = jnp.zeros(MM3.shape, F32)
    VT3[...] = jnp.zeros(VT3.shape, BF)
    AM3[...] = jnp.zeros(AM3.shape, F32)
    for c in range(8):
        HB[c, pl.ds(0, 8), :] = jnp.zeros((8, 128), F32)
        HB[c, pl.ds(8 + S, 8), :] = jnp.zeros((8, 128), F32)

    def ln_a(r0, n, gate=None):
        xf = ln(tok1(xb[pl.ds(r0, n), :].astype(F32), gate))
        t = None
        for cb in range(8):
            v = xf[:, cb * 128:(cb + 1) * 128]
            XN[cb, pl.ds(r0, n), :] = v.astype(BF)
            t = v if t is None else jnp.maximum(t, v)
        return jnp.max(t.reshape(n // 8, 8, 128), axis=0)

    x_copy(0).wait()

    def ln0(t, c):
        ln_a(pl.multiple_of(t * 128, 128), 128)
        return c
    lax.fori_loop(0, L // 128, ln0, 0)

    def xn_tile(r0, n):
        return cat([ld(XN, cb, (r0, n)) for cb in range(8)], 1)

    def a_segment(it, s):
        r0 = pl.multiple_of(s * L, L)
        first = jnp.logical_and(it == 0, s == 0)
        st = {}

        def gate(name, v, n):
            st['gate', name + '0'] = v[0:8, 0:128]
            st['gate', name + '1'] = v[n - 8:n, 0:128]

        def proj_k(g, t, gi):
            xn = xn_tile(r0 + 128 * t, 128)
            k = mm(xn, ld(wk, gi, None))
            st['K', g, t] = k.astype(BF)
            gate('prev', k, 128)
            pk = phi(k)
            st['PK', g, t] = pk
            zs = jnp.sum(pk.reshape(16, 8, 128), axis=0)
            st['z', g] = zs if t == 0 else st['z', g] + zs

        def proj_qv(g, t, gi):
            xn = xn_tile(r0 + 128 * t, 128)
            wqv = jnp.concatenate([ld(wq, gi, None), ld(wv, gi, None)], axis=1)
            r = mm(wqv, xn, TT)
            q = r[:128]
            gate('prev', r, 256)
            st['QT', g, t] = q * QSCALE
            st['PQT', g, t] = phi(q)
            st['VT', g, t] = r[128:].astype(BF)

        def qk(g, i, j):
            qt = st['QT', g, i]
            z32 = jnp.zeros((32, 128), F32)
            w = jnp.concatenate([jnp.concatenate([qt[32 * hh:32 * hh + 32] if rr == hh else z32 for rr in range(4)], axis=0)
                                 for hh in range(4)], axis=1).astype(BF)
            s_ = mm(st['K', g, j], w)
            gate('prev', s_, 128)
            if i == j:
                s_ = s_ + jnp.concatenate([bias[...]] * 4, axis=1)
            if g == NG - 1 and i == 3:
                SS[j] = s_
            else:
                st['s', g, i, j] = s_
            mx = jnp.max(s_.reshape(16, 8, 512), axis=0)
            st['m', g, i] = mx if j == 0 else jnp.maximum(st['m', g, i], mx)

        def sm(g, i, j, gt=None):
            if j == 0:
                m8 = st['m', g, i] if g != 'c' else MM3[...]
                st['mr', g, i] = jnp.broadcast_to(jnp.max(m8, axis=0, keepdims=True), (8, 512))
            m = tok(st['mr', g, i], st['gate', gt] if gt else None)
            s_ = st.pop(('s', g, i, j)) if g != 'c' else SS[j]
            ps = []
            for c in range(8):
                e0 = jnp.exp2(s_[16 * c:16 * c + 8] - m)
                e1 = jnp.exp2(s_[16 * c + 8:16 * c + 16] - m)
                ee = e0 + e1
                st['l', g, i] = ee if (j == 0 and c == 0) else st['l', g, i] + ee
                ps.append(e0); ps.append(e1)
            st['p', g, i, j] = jnp.concatenate(ps, axis=0)

        def pv(g, i, j):
            pb = st.pop(('p', g, i, j))
            for hh in range(4):
                vt = st['VT', g, j][32 * hh:32 * hh + 32] if g != 'c' else ld(VT3, j, (32 * hh, 32))
                ot = mm(vt, pb[:, 128 * hh:128 * (hh + 1)].astype(BF))
                st['o', g, i, hh] = ot if j == 0 else st['o', g, i, hh] + ot

        def memrd(g, gi):
            pq = cat([st['PQT', g, t] for t in range(4)], 1).astype(BF)
            mem = mm(ld(A, gi, None), pq)
            gate('prev', mem, 160)
            for hh in range(4):
                g1 = Gt[gi * 4 + hh][0:1, :]
                den = mem[40 * hh + 32:40 * hh + 33, :] + 1e-6
                wm = g1[:, 0:1] / den
                st['AM', g, hh] = mem[40 * hh:40 * hh + 32, :] * wm

        def fin(g, i, gi):
            l = jnp.sum(st['l', g, i], axis=0, keepdims=True)
            os_ = []
            for hh in range(4):
                g1 = Gt[gi * 4 + hh][0:1, :]
                wd = (1.0 - g1) / l[:, 128 * hh:128 * (hh + 1)]
                am = st['AM', g, hh][:, 128 * i:128 * (i + 1)] if g != 'c' else AM3[pl.ds(32 * hh, 32), :]
                os_.append(st['o', g, i, hh] * wd + am)
            OT[gi, i] = jnp.concatenate(os_, axis=0).astype(BF)

        def save_tail(g):
            for j in range(4):
                VT3[j] = st['VT', g, j]
            MM3[...] = st['m', g, 3]
            for hh in range(4):
                AM3[pl.ds(32 * hh, 32), :] = st['AM', g, hh][:, 384:512]

        def upd(g, gi):
            pk = cat([st['PK', g, t] for t in range(4)], 0).astype(BF)
            d = mm(cat([st['VT', g, t] for t in range(4)], 1), pk)
            gate('prev', d, 128)
            mt = MT[gi] + jnp.where(blk, d, 0.0)
            MT[gi] = mt
            z = Z[gi] + jnp.broadcast_to(jnp.sum(st['z', g], axis=0, keepdims=True), (8, 128))
            Z[gi] = z
            lh = lax.broadcasted_iota(I32, (8, 128), 1) // DH
            parts = []
            for hh in range(4):
                parts.append(mt[32 * hh:32 * hh + 32, :])
                parts.append(jnp.where(lh == hh, z, 0.0))
            A[gi] = jnp.concatenate(parts, axis=0).astype(BF)

        def group(g, gi, p, pi):
            proj_k(g, 0, gi)
            sm(p, 3, 0)
            sm(p, 3, 1, 'prev0'); pv(p, 3, 0)
            proj_qv(g, 0, gi)
            sm(p, 3, 2, 'prev1'); pv(p, 3, 1)
            qk(g, 0, 0)
            proj_k(g, 1, gi)
            sm(p, 3, 3, 'prev0'); pv(p, 3, 2)
            proj_qv(g, 1, gi)
            sm(g, 0, 0, 'prev0')
            pv(p, 3, 3); fin(p, 3, pi)
            qk(g, 1, 0)
            qk(g, 1, 1)
            sm(g, 1, 0)
            pv(g, 0, 0)
            proj_k(g, 2, gi)
            pv(g, 1, 0)
            proj_qv(g, 2, gi)
            sm(g, 1, 1, 'prev0')
            qk(g, 2, 0)
            pv(g, 1, 1)
            qk(g, 2, 1)
            qk(g, 2, 2)
            sm(g, 2, 0)
            proj_k(g, 3, gi)
            pv(g, 2, 0)
            proj_qv(g, 3, gi)
            sm(g, 2, 1, 'prev0')
            memrd(g, gi)
            pv(g, 2, 1)
            qk(g, 3, 0)
            sm(g, 2, 2, 'prev0')
            qk(g, 3, 1)
            qk(g, 3, 2)
            pv(g, 2, 2)
            fin(g, 0, gi); fin(g, 1, gi); fin(g, 2, gi)
            qk(g, 3, 3)
            upd(g, gi)

        def gl(k, c):
            g0 = k * NG

            @pl.when(first)
            def _():
                for g in range(NG):
                    for cp in qkv_copies(g0 + g):
                        cp.wait()

                @pl.when(k == 0)
                def _():
                    start_batch2()

            for g in range(NG):
                if g == 0:
                    group(g, g0, 'c', (g0 + G - 1) % G)
                else:
                    group(g, g0 + g, g - 1, g0 + g - 1)
            save_tail(NG - 1)
            return c
        lax.fori_loop(0, G // NG, gl, 0)
        st.clear()

        @pl.when(first)
        def _():
            wait("wo")
            wait("w1")
            start_batch3()

        sn = jnp.minimum(s + 1, NSEG - 1)

        @pl.when(jnp.logical_and(it == 0, s < NSEG - 1))
        def _():
            x_copy(sn).wait()

        pend = []

        def drain(acc):
            for e in pend:
                e[0] -= 1
            ready = [e[1] for e in pend if e[0] <= 0]
            pend[:] = [e for e in pend if e[0] > 0]
            for t in ready:
                acc = inject(acc, [(0, t)])
            return acc

        def aout(i, fill=()):
            rows = pl.ds(r0 + 128 * i, 128)
            ot = cat([ld(OT, g, i, None) for g in range(G)], 0)
            xs = []
            for n in range(8):
                acc = mm(ot, ld(wo, n, None), TN)
                acc = drain(acc)
                if n < len(fill) and fill[n] is not None:
                    fill[n](acc[0:8])
                xs.append(acc)
            x = xb[rows, :].astype(F32) + cat(xs, 1)
            X[rows, :] = x
            st['x', i] = x

        def lnb(i, c):
            def f(gate):
                rows = pl.ds(r0 + 128 * i + 32 * c, 32)
                xn, xnn = ln2(tok1(st['x', i][32 * c:32 * c + 32], gate))
                XF[rows, :] = xn
                st['xnn', i, c] = xnn
            return f

        def lna(c):
            def f(gate):
                pend.append([2, ln_a(pl.multiple_of(sn * L + 64 * c, 64), 64, gate)])
            return f

        def hproj(i, fill=()):
            xnn = cat([st['xnn', i, c] for c in range(4)], 0).astype(BF)
            for n in range(8):
                acc = mm(xnn, ld(w1, n, None))
                acc = drain(acc)
                if n < len(fill) and fill[n] is not None:
                    fill[n](acc[0:8])
                HB[n, pl.ds(pl.multiple_of(r0 + 128 * i + 8, 8), 128), :] = gelu(acc)

        p = 'c'

        def psm(j):
            def f(gate):
                st['gate', 'x'] = gate
                sm(p, 3, j, 'x')
            return f

        def lnbs(i):
            return [lnb(i, 0), lnb(i, 1), lnb(i, 2), None, lnb(i, 3)]

        aout(0, [psm(0), lna(0), None, psm(1), lna(1), None, psm(2), lna(2)])
        pv(p, 3, 0); pv(p, 3, 1)
        aout(1, lnbs(0))
        pv(p, 3, 2)
        hproj(0, lnbs(1))
        aout(2, [psm(3), lna(3), None, lna(4), None, lna(5)])
        pv(p, 3, 3); fin(p, 3, G - 1)
        hproj(1, lnbs(2))
        aout(3, [lna(6), None, None, lna(7)])
        hproj(2, lnbs(3))
        hproj(3)

    def layer(it, carry):
        MT[...] = jnp.zeros(MT.shape, F32)
        Z[...] = jnp.zeros(Z.shape, F32)
        A[...] = jnp.zeros(A.shape, BF)

        def seg(s, c):
            a_segment(it, s)
            return c
        lax.fori_loop(0, NSEG, seg, 0)

        @pl.when(it == 0)
        def _():
            for n in ("w2", "w3", "w4"):
                wait(n)

        def b2(t, c):
            r0 = pl.multiple_of(t * TM, TM)
            sh = [-1, -1, 1, 1, -2, -2, 2, 2]
            HM = TM // 2
            x1 = []
            u = []
            for a in range(2):
                ra = r0 + a * HM
                hsft = jnp.concatenate([HB[cb, pl.ds(ra + (8 + sh[cb]), HM), :].astype(BF) for cb in range(8)], axis=1)
                x1.append(XF[pl.ds(ra, HM), :] + mm(hsft, full(w2)))
            tp = (t + (S // TM) - 2) % (S // TM)
            x1h = [ln(x1[a]).astype(BF) for a in range(2)]
            NH = 4
            pre0 = cat([mm(x1h[a], full(w3, cols=range(NH))) for a in range(2)], 0)
            pre = cat([pre0, mm(cat(x1h, 0), full(w3, cols=range(NH, NF)))], 1)
            toks = []
            for cch in range(4):
                g = pre[0:8, 128 * (5 * cch + 7):128 * (5 * cch + 8)]
                toks.append((5 * cch + 12, ln_a(pl.multiple_of(tp * TM + cch * 64, 64), 64, g)))
            u = gelu(inject(pre, toks)).astype(BF)
            y = mm(u, full(w4))
            xnew = X[pl.ds(r0, TM), :] + cat(x1, 0) + y
            xb[pl.ds(r0, TM), :] = xnew.astype(BF)

            @pl.when(it == 1)
            def _():
                out_copy(t).start()
            return c
        lax.fori_loop(0, S // TM, b2, 0)
        return carry

    lax.fori_loop(0, 2, layer, 0)
    for t in range(S // TM):
        out_copy(t).wait()


@jax.jit
def pallas_interleave_layers__memory_aug_infini_attn__mixer_s_mlp__prompt_kernel(
        A_x, A_wq, A_wk, A_wv, A_wo, A_beta, B_x, B_w1, B_w2, B_w3, B_w4):
    anyspec = pl.BlockSpec(memory_space=pl.ANY)
    V = pltpu.VMEM
    wsq = V((G, D, 128), BF)
    dma = pltpu.SemaphoreType.DMA
    out = pl.pallas_call(
        kernel,
        out_shape=jax.ShapeDtypeStruct((S, D), BF),
        in_specs=[anyspec] * 5 + [pl.BlockSpec(memory_space=pltpu.VMEM)] + [anyspec] * 4,
        out_specs=anyspec,
        scratch_shapes=[
            wsq, wsq, wsq, wsq, wsq, wsq,
            V((NF, D, 128), BF), V((G, F, 128), BF),
            V((S, D), BF),
            V((S, D), F32),
            V((S, D), F32),
            V((G, S, 128), BF),
            V((G, 128, 128), F32),
            V((G, 8, 128), F32),
            V((G, 160, 128), BF),
            V((8, S + 16, 128), F32),
            V((H, 8, 128), F32),
            V((128, 128), F32),
            V((4, 128, 512), F32),
            V((8, 512), F32),
            V((4, 128, 128), BF),
            V((128, 128), F32),
            V((G, 4, 128, 128), BF),
            dma((NSEG,)), dma((G,)), dma((G,)), dma((G,)), dma((5,)), dma((S // TM,)),
        ],
        compiler_params=pltpu.CompilerParams(vmem_limit_bytes=118 * 1024 * 1024),
        name="mykern",
    )(A_x.reshape(S, D), A_wq, A_wk, A_wv, A_wo, A_beta.reshape(1, H), B_w1, B_w2, B_w3, B_w4)
    return out.reshape(1, S, D)
```

```python
import functools
import math

import jax
import jax.numpy as jnp
from jax import lax
import jax.experimental.pallas as pl
import jax.experimental.pallas.tpu as pltpu

S, D, H, DH, NSEG, L, F = 2048, 1024, 32, 32, 4, 512, 3584
G = 8
NG = 4
NF = F // 128
TM = 256
LOG2E = 1.4426950408889634
QSCALE = DH ** -0.5 * LOG2E
NEG = -1e9 * LOG2E
BF = jnp.bfloat16
F32 = jnp.float32
I32 = jnp.int32

NN = (((1,), (0,)), ((), ()))
TN = (((0,), (0,)), ((), ()))
TT = (((0,), (1,)), ((), ()))


def mm(a, b, dn=NN):
    return lax.dot_general(a, b, dn, preferred_element_type=F32)


def ld(ref, *idx):
    *lead, rows = idx
    if rows is None:
        v = ref.bitcast(I32)[tuple(lead)]
    else:
        st, n = rows
        st2 = st // 2 if isinstance(st, int) else pl.multiple_of(st // 2, 8)
        v = ref.bitcast(I32)[(*lead, pl.ds(st2, n // 2), slice(None))]
    return pltpu.bitcast(v, BF)


def cat(xs, axis):
    return jnp.concatenate(xs, axis=axis) if len(xs) > 1 else xs[0]


def ln(x):
    m = jnp.mean(x, axis=-1, keepdims=True)
    d = x - m
    v = jnp.mean(d * d, axis=-1, keepdims=True)
    return d * lax.rsqrt(v + 1e-5)


def ln2(x):
    m = jnp.mean(x, axis=-1, keepdims=True)
    d = x - m
    v = jnp.mean(d * d, axis=-1, keepdims=True)
    r = lax.rsqrt(v + 1e-5)
    r2 = lax.rsqrt(v * r * r + 1e-5)
    return d * r, d * (r * r2)


def gelu(x):
    c0 = math.sqrt(2.0 / math.pi)
    u = x * (x * x * (c0 * 0.044715) + c0)
    hx = 0.5 * x
    return hx * jnp.tanh(u) + hx


def phi(t):
    return jnp.where(t > 0, t + 1.0, jnp.exp(t))


def tok(x, gate):
    if gate is None:
        return x
    t = gate * 0.0
    if x.shape[0] != 8:
        t = cat([t] * (x.shape[0] // 8), 0)
    return x + cat([t] * (x.shape[1] // 128), 1)


def tok1(x, gate):
    if gate is None:
        return x
    return cat([tok(x[:, 0:128], gate), x[:, 128:]], 1)


def inject(v, toks):
    if not toks:
        return v
    d = dict(toks)
    top = cat([v[0:8, 128 * c:128 * (c + 1)] + d[c] * 0.0 if c in d else v[0:8, 128 * c:128 * (c + 1)]
               for c in range(v.shape[1] // 128)], 1)
    return cat([top, v[8:]], 0) if v.shape[0] > 8 else top


def kernel(x_hbm, wq_hbm, wk_hbm, wv_hbm, wo_hbm, beta_ref, w1_hbm, w2_hbm, w3_hbm, w4_hbm,
           out_hbm,
           wq, wk, wv, wo, w1, w2, w3, w4,
           xb, X, XF, XN, MT, Z, A, HB, Gt, bias, SS, MM3, VT3, AM3, OT,
           sx, sq, sk, sv, sw, so):
    def x_copy(s):
        return pltpu.make_async_copy(x_hbm.at[pl.ds(s * L, L), :], xb.at[pl.ds(s * L, L), :], sx.at[s])

    def qkv_copies(g):
        c0 = g * 128 if isinstance(g, int) else pl.multiple_of(g * 128, 128)
        return [pltpu.make_async_copy(src.at[:, pl.ds(c0, 128)], dst.at[g], sem.at[g])
                for src, dst, sem in ((wk_hbm, wk, sk), (wq_hbm, wq, sq), (wv_hbm, wv, sv))]

    def w_copies(i, src, dst):
        return [pltpu.make_async_copy(src.at[:, pl.ds(c * 128, 128)], dst.at[c], sw.at[i]) for c in range(dst.shape[0])]

    def out_copy(t):
        r0 = t * TM if isinstance(t, int) else pl.multiple_of(t * TM, TM)
        return pltpu.make_async_copy(xb.at[pl.ds(r0, TM), :], out_hbm.at[pl.ds(r0, TM), :], so.at[t])

    wl = {"wo": (0, wo_hbm, wo), "w1": (1, w1_hbm, w1), "w2": (2, w2_hbm, w2), "w3": (3, w3_hbm, w3), "w4": (4, w4_hbm, w4)}
    x_copy(0).start()
    for g in range(NG):
        for cp in qkv_copies(g):
            cp.start()

    def start_batch2():
        for g in range(NG, G):
            for cp in qkv_copies(g):
                cp.start()
        for n in ("wo", "w1"):
            for cp in w_copies(*wl[n]):
                cp.start()
        x_copy(1).start()

    def start_batch3():
        for s in range(2, NSEG):
            x_copy(s).start()
        for n in ("w2", "w3", "w4"):
            for cp in w_copies(*wl[n]):
                cp.start()

    def wait(n):
        for cp in w_copies(*wl[n]):
            cp.wait()

    def full(w, k0=0, k1=None, cols=None):
        k1 = w.shape[1] if k1 is None else k1
        cols = range(w.shape[0]) if cols is None else cols
        return cat([ld(w, c, (k0, k1 - k0)) for c in cols], 1)

    r = lax.broadcasted_iota(I32, (128, 128), 0)
    c = lax.broadcasted_iota(I32, (128, 128), 1)
    bias[...] = jnp.where(r > c, NEG, 0.0).astype(F32)
    blk = (lax.broadcasted_iota(I32, (128, 128), 0) // DH) == (lax.broadcasted_iota(I32, (128, 128), 1) // DH)

    b = beta_ref[...].astype(F32)
    gv = jax.nn.sigmoid(b)
    rr = lax.broadcasted_iota(I32, (H, H), 0)
    cc = lax.broadcasted_iota(I32, (H, H), 1)
    col = jnp.sum(jnp.where(rr == cc, jnp.broadcast_to(gv, (H, H)), 0.0), axis=1, keepdims=True)
    gb = jnp.broadcast_to(col, (H, 128))
    for h in range(H):
        Gt[h] = jnp.broadcast_to(gb[h:h + 1, :], (8, 128))
    SS[...] = jnp.zeros(SS.shape, F32)
    MM3[...] = jnp.zeros(MM3.shape, F32)
    VT3[...] = jnp.zeros(VT3.shape, BF)
    AM3[...] = jnp.zeros(AM3.shape, F32)
    for c in range(8):
        HB[c, pl.ds(0, 8), :] = jnp.zeros((8, 128), F32)
        HB[c, pl.ds(8 + S, 8), :] = jnp.zeros((8, 128), F32)

    def ln_a(r0, n, gate=None):
        xf = ln(tok1(xb[pl.ds(r0, n), :].astype(F32), gate))
        t = None
        for cb in range(8):
            v = xf[:, cb * 128:(cb + 1) * 128]
            XN[cb, pl.ds(r0, n), :] = v.astype(BF)
            t = v if t is None else jnp.maximum(t, v)
        return jnp.max(t.reshape(n // 8, 8, 128), axis=0)

    x_copy(0).wait()

    def ln0(t, c):
        ln_a(pl.multiple_of(t * 128, 128), 128)
        return c
    lax.fori_loop(0, L // 128, ln0, 0)

    def xn_tile(r0, n):
        return cat([ld(XN, cb, (r0, n)) for cb in range(8)], 1)

    def a_segment(it, s):
        r0 = pl.multiple_of(s * L, L)
        first = jnp.logical_and(it == 0, s == 0)
        st = {}

        def gate(name, v, n):
            st['gate', name + '0'] = v[0:8, 0:128]
            st['gate', name + '1'] = v[n - 8:n, 0:128]

        def proj_k(g, t, gi):
            xn = xn_tile(r0 + 128 * t, 128)
            k = mm(xn, ld(wk, gi, None))
            st['K', g, t] = k.astype(BF)
            gate('prev', k, 128)
            pk = phi(k)
            st['PK', g, t] = pk
            zs = jnp.sum(pk.reshape(16, 8, 128), axis=0)
            st['z', g] = zs if t == 0 else st['z', g] + zs

        def proj_qv(g, t, gi):
            xn = xn_tile(r0 + 128 * t, 128)
            wqv = jnp.concatenate([ld(wq, gi, None), ld(wv, gi, None)], axis=1)
            r = mm(wqv, xn, TT)
            q = r[:128]
            gate('prev', r, 256)
            st['QT', g, t] = q * QSCALE
            st['PQT', g, t] = phi(q)
            st['VT', g, t] = r[128:]
            for hh in range(4):
                st['VH', g, t, hh] = r[128 + 32 * hh:160 + 32 * hh].astype(BF)

        def qk(g, i, j):
            qt = st['QT', g, i]
            z32 = jnp.zeros((32, 128), F32)
            w = jnp.concatenate([jnp.concatenate([qt[32 * hh:32 * hh + 32] if rr == hh else z32 for rr in range(4)], axis=0)
                                 for hh in range(4)], axis=1).astype(BF)
            s_ = mm(st['K', g, j], w)
            gate('prev', s_, 128)
            if i == j:
                s_ = s_ + jnp.concatenate([bias[...]] * 4, axis=1)
            if g == NG - 1 and i == 3:
                SS[j] = s_
            else:
                st['s', g, i, j] = s_
            mx = jnp.max(s_.reshape(16, 8, 512), axis=0)
            st['m', g, i] = mx if j == 0 else jnp.maximum(st['m', g, i], mx)

        def sm(g, i, j, gt=None):
            if j == 0:
                m8 = st['m', g, i] if g != 'c' else MM3[...]
                st['mr', g, i] = jnp.broadcast_to(jnp.max(m8, axis=0, keepdims=True), (8, 512))
            m = tok(st['mr', g, i], st['gate', gt] if gt else None)
            s_ = st.pop(('s', g, i, j)) if g != 'c' else SS[j]
            ps = []
            for c in range(8):
                e0 = jnp.exp2(s_[16 * c:16 * c + 8] - m)
                e1 = jnp.exp2(s_[16 * c + 8:16 * c + 16] - m)
                ee = e0 + e1
                st['l', g, i] = ee if (j == 0 and c == 0) else st['l', g, i] + ee
                ps.append(e0); ps.append(e1)
            st['p', g, i, j] = jnp.concatenate(ps, axis=0)

        def pv(g, i, j):
            pb = st.pop(('p', g, i, j))
            for hh in range(4):
                vt = st['VH', g, j, hh] if g != 'c' else ld(VT3, j, (32 * hh, 32))
                ot = mm(vt, pb[:, 128 * hh:128 * (hh + 1)].astype(BF))
                st['o', g, i, hh] = ot if j == 0 else st['o', g, i, hh] + ot

        def memrd(g, gi):
            pq = cat([st['PQT', g, t] for t in range(4)], 1).astype(BF)
            mem = mm(ld(A, gi, None), pq)
            gate('prev', mem, 160)
            for hh in range(4):
                g1 = Gt[gi * 4 + hh][0:1, :]
                den = mem[40 * hh + 32:40 * hh + 33, :] + 1e-6
                wm = g1[:, 0:1] / den
                st['AM', g, hh] = mem[40 * hh:40 * hh + 32, :] * wm

        def fin(g, i, gi):
            l = jnp.sum(st['l', g, i], axis=0, keepdims=True)
            os_ = []
            for hh in range(4):
                g1 = Gt[gi * 4 + hh][0:1, :]
                wd = (1.0 - g1) / l[:, 128 * hh:128 * (hh + 1)]
                am = st['AM', g, hh][:, 128 * i:128 * (i + 1)] if g != 'c' else AM3[pl.ds(32 * hh, 32), :]
                os_.append(st['o', g, i, hh] * wd + am)
            OT[gi, i] = jnp.concatenate(os_, axis=0).astype(BF)

        def save_tail(g):
            for j in range(4):
                VT3[j] = st['VT', g, j].astype(BF)
            MM3[...] = st['m', g, 3]
            for hh in range(4):
                AM3[pl.ds(32 * hh, 32), :] = st['AM', g, hh][:, 384:512]

        def upd(g, gi):
            pk = cat([st['PK', g, t] for t in range(4)], 0).astype(BF)
            d = mm(cat([st['VT', g, t] for t in range(4)], 1).astype(BF), pk)
            gate('prev', d, 128)
            mt = MT[gi] + jnp.where(blk, d, 0.0)
            MT[gi] = mt
            z = Z[gi] + jnp.broadcast_to(jnp.sum(st['z', g], axis=0, keepdims=True), (8, 128))
            Z[gi] = z
            lh = lax.broadcasted_iota(I32, (8, 128), 1) // DH
            parts = []
            for hh in range(4):
                parts.append(mt[32 * hh:32 * hh + 32, :])
                parts.append(jnp.where(lh == hh, z, 0.0))
            A[gi] = jnp.concatenate(parts, axis=0).astype(BF)

        def group(g, gi, p, pi):
            proj_k(g, 0, gi)
            sm(p, 3, 0)
            sm(p, 3, 1, 'prev0'); pv(p, 3, 0)
            proj_qv(g, 0, gi)
            sm(p, 3, 2, 'prev1'); pv(p, 3, 1)
            qk(g, 0, 0)
            proj_k(g, 1, gi)
            sm(p, 3, 3, 'prev0'); pv(p, 3, 2)
            proj_qv(g, 1, gi)
            sm(g, 0, 0, 'prev0')
            pv(p, 3, 3); fin(p, 3, pi)
            qk(g, 1, 0)
            qk(g, 1, 1)
            sm(g, 1, 0)
            pv(g, 0, 0)
            proj_k(g, 2, gi)
            pv(g, 1, 0)
            proj_qv(g, 2, gi)
            sm(g, 1, 1, 'prev0')
            qk(g, 2, 0)
            pv(g, 1, 1)
            qk(g, 2, 1)
            qk(g, 2, 2)
            sm(g, 2, 0)
            proj_k(g, 3, gi)
            pv(g, 2, 0)
            proj_qv(g, 3, gi)
            sm(g, 2, 1, 'prev0')
            memrd(g, gi)
            pv(g, 2, 1)
            qk(g, 3, 0)
            sm(g, 2, 2, 'prev0')
            qk(g, 3, 1)
            qk(g, 3, 2)
            pv(g, 2, 2)
            fin(g, 0, gi); fin(g, 1, gi); fin(g, 2, gi)
            qk(g, 3, 3)
            upd(g, gi)

        def gl(k, c):
            g0 = k * NG

            @pl.when(first)
            def _():
                for g in range(NG):
                    for cp in qkv_copies(g0 + g):
                        cp.wait()

                @pl.when(k == 0)
                def _():
                    start_batch2()

            for g in range(NG):
                if g == 0:
                    group(g, g0, 'c', (g0 + G - 1) % G)
                else:
                    group(g, g0 + g, g - 1, g0 + g - 1)
            save_tail(NG - 1)
            return c
        lax.fori_loop(0, G // NG, gl, 0)
        st.clear()

        @pl.when(first)
        def _():
            wait("wo")
            wait("w1")
            start_batch3()

        sn = jnp.minimum(s + 1, NSEG - 1)

        @pl.when(jnp.logical_and(it == 0, s < NSEG - 1))
        def _():
            x_copy(sn).wait()

        pend = []

        def drain(acc):
            for e in pend:
                e[0] -= 1
            ready = [e[1] for e in pend if e[0] <= 0]
            pend[:] = [e for e in pend if e[0] > 0]
            for t in ready:
                acc = inject(acc, [(0, t)])
            return acc

        def aout(i, fill=()):
            rows = pl.ds(r0 + 128 * i, 128)
            ot = cat([ld(OT, g, i, None) for g in range(G)], 0)
            xs = []
            for n in range(8):
                acc = mm(ot, ld(wo, n, None), TN)
                acc = drain(acc)
                if n < len(fill) and fill[n] is not None:
                    fill[n](acc[0:8])
                xs.append(acc)
            x = xb[rows, :].astype(F32) + cat(xs, 1)
            X[rows, :] = x
            st['x', i] = x

        def lnb(i, c):
            def f(gate):
                rows = pl.ds(r0 + 128 * i + 32 * c, 32)
                xn, xnn = ln2(tok1(st['x', i][32 * c:32 * c + 32], gate))
                XF[rows, :] = xn
                st['xnn', i, c] = xnn
            return f

        def lna(c):
            def f(gate):
                pend.append([2, ln_a(pl.multiple_of(sn * L + 64 * c, 64), 64, gate)])
            return f

        def hproj(i, fill=()):
            xnn = cat([st['xnn', i, c] for c in range(4)], 0).astype(BF)
            for n in range(8):
                acc = mm(xnn, ld(w1, n, None))
                acc = drain(acc)
                if n < len(fill) and fill[n] is not None:
                    fill[n](acc[0:8])
                HB[n, pl.ds(pl.multiple_of(r0 + 128 * i + 8, 8), 128), :] = gelu(acc)

        p = 'c'

        def psm(j):
            def f(gate):
                st['gate', 'x'] = gate
                sm(p, 3, j, 'x')
            return f

        def lnbs(i):
            return [lnb(i, 0), lnb(i, 1), lnb(i, 2), None, lnb(i, 3)]

        aout(0, [psm(0), lna(0), None, psm(1), lna(1), None, psm(2), lna(2)])
        pv(p, 3, 0); pv(p, 3, 1)
        aout(1, lnbs(0))
        pv(p, 3, 2)
        hproj(0, lnbs(1))
        aout(2, [psm(3), lna(3), None, lna(4), None, lna(5)])
        pv(p, 3, 3); fin(p, 3, G - 1)
        hproj(1, lnbs(2))
        aout(3, [lna(6), None, None, lna(7)])
        hproj(2, lnbs(3))
        hproj(3)

    def layer(it, carry):
        MT[...] = jnp.zeros(MT.shape, F32)
        Z[...] = jnp.zeros(Z.shape, F32)
        A[...] = jnp.zeros(A.shape, BF)

        def seg(s, c):
            a_segment(it, s)
            return c
        lax.fori_loop(0, NSEG, seg, 0)

        @pl.when(it == 0)
        def _():
            for n in ("w2", "w3", "w4"):
                wait(n)

        def b2(t, c):
            r0 = pl.multiple_of(t * TM, TM)
            sh = [-1, -1, 1, 1, -2, -2, 2, 2]
            HM = TM // 2
            x1 = []
            u = []
            for a in range(2):
                ra = r0 + a * HM
                hsft = jnp.concatenate([HB[cb, pl.ds(ra + (8 + sh[cb]), HM), :].astype(BF) for cb in range(8)], axis=1)
                x1.append(XF[pl.ds(ra, HM), :] + mm(hsft, full(w2)))
            tp = (t + (S // TM) - 2) % (S // TM)
            x1h = [ln(x1[a]).astype(BF) for a in range(2)]
            NH = 4
            pre0 = cat([mm(x1h[a], full(w3, cols=range(NH))) for a in range(2)], 0)
            pre = cat([pre0, mm(cat(x1h, 0), full(w3, cols=range(NH, NF)))], 1)
            toks = []
            for cch in range(4):
                g = pre[0:8, 128 * (5 * cch + 7):128 * (5 * cch + 8)]
                toks.append((5 * cch + 12, ln_a(pl.multiple_of(tp * TM + cch * 64, 64), 64, g)))
            u = gelu(inject(pre, toks)).astype(BF)
            y = mm(u, full(w4))
            xnew = X[pl.ds(r0, TM), :] + cat(x1, 0) + y
            xb[pl.ds(r0, TM), :] = xnew.astype(BF)

            @pl.when(it == 1)
            def _():
                out_copy(t).start()
            return c
        lax.fori_loop(0, S // TM, b2, 0)
        return carry

    lax.fori_loop(0, 2, layer, 0)
    for t in range(S // TM):
        out_copy(t).wait()


@jax.jit
def pallas_interleave_layers__memory_aug_infini_attn__mixer_s_mlp__prompt_kernel(
        A_x, A_wq, A_wk, A_wv, A_wo, A_beta, B_x, B_w1, B_w2, B_w3, B_w4):
    anyspec = pl.BlockSpec(memory_space=pl.ANY)
    V = pltpu.VMEM
    wsq = V((G, D, 128), BF)
    dma = pltpu.SemaphoreType.DMA
    out = pl.pallas_call(
        kernel,
        out_shape=jax.ShapeDtypeStruct((S, D), BF),
        in_specs=[anyspec] * 5 + [pl.BlockSpec(memory_space=pltpu.VMEM)] + [anyspec] * 4,
        out_specs=anyspec,
        scratch_shapes=[
            wsq, wsq, wsq, wsq, wsq, wsq,
            V((NF, D, 128), BF), V((G, F, 128), BF),
            V((S, D), BF),
            V((S, D), F32),
            V((S, D), F32),
            V((G, S, 128), BF),
            V((G, 128, 128), F32),
            V((G, 8, 128), F32),
            V((G, 160, 128), BF),
            V((8, S + 16, 128), F32),
            V((H, 8, 128), F32),
            V((128, 128), F32),
            V((4, 128, 512), F32),
            V((8, 512), F32),
            V((4, 128, 128), BF),
            V((128, 128), F32),
            V((G, 4, 128, 128), BF),
            dma((NSEG,)), dma((G,)), dma((G,)), dma((G,)), dma((5,)), dma((S // TM,)),
        ],
        compiler_params=pltpu.CompilerParams(vmem_limit_bytes=118 * 1024 * 1024),
        name="mykern",
    )(A_x.reshape(S, D), A_wq, A_wk, A_wv, A_wo, A_beta.reshape(1, H), B_w1, B_w2, B_w3, B_w4)
    return out.reshape(1, S, D)
```
